```python
import jax
import jax.numpy as jnp

def _softmax(x, axis=-1):
    return jax.nn.softmax(x, axis=axis)

def _gelu(x):
    return jax.nn.gelu(x, approximate=True)

def _silu(x):
    return jax.nn.silu(x)

def _sigmoid(x):
    return jax.nn.sigmoid(x)

def _layernorm(x, axis=-1, eps=1e-05):
    m = jnp.mean(x, axis=axis, keepdims=True)
    v = jnp.var(x, axis=axis, keepdims=True)
    return (x - m) / jnp.sqrt(v + eps)

def _scatter_add(tgt, idx, src, axis=0):
    return tgt.at[idx].add(src)

def _segment_sum(src, seg, n):
    return jax.ops.segment_sum(src, seg, n)

class _Rng:

    def __init__(self, key):
        self._k = key

    def _next(self):
        self._k, sub = jax.random.split(self._k)
        return sub

    def normal(self, shape):
        return jax.random.normal(self._next(), shape, dtype=jnp.bfloat16)

    def randint(self, lo, hi, shape):
        return jax.random.randint(self._next(), shape, lo, hi, dtype=jnp.int32)

    def uniform(self, shape, lo=0.0, hi=1.0):
        return jax.random.uniform(self._next(), shape, jnp.bfloat16, lo, hi)

    def permutation(self, n):
        return jax.random.permutation(self._next(), n)
kernel_name = 'interleave_layers__linear_kernel_hedgehog__mixer_gmlp__prompt'

def _fwd_setup_inputs():
    _rng = _Rng(jax.random.key(int.from_bytes(__import__("os").urandom(4), "little")))
    _w = lambda a: (lambda t: t.astype(jnp.bfloat16) if jnp.issubdtype(t.dtype, jnp.floating) else t)(jnp.asarray(a))

    def _A_setup():
        B, S, D, H = (1, 2048, 640, 32)
        Dh = D // H
        return {'x': _w((lambda *s: _rng.normal(s) * 0.05)(B, S, D)), 'wqkv': _w((lambda *s: _rng.normal(s) * 0.05)(D, 3 * D)), 'w_phi': _w((lambda *s: _rng.normal(s) * 0.05)(H, Dh, Dh) * Dh ** (-0.5)), 'wo': _w((lambda *s: _rng.normal(s) * 0.05)(D, D))}
    _A_in = _A_setup()

    def _B_setup():
        B, S, D, F = (1, 2048, 640, 1536)
        Fh = F // 2
        return {'x': _w((lambda *s: _rng.normal(s) * 0.05)(B, S, D)), 'w_in': _w((lambda *s: _rng.normal(s) * 0.05)(D, 2 * Fh)), 'w_sp': _w(0.01 * (lambda *s: _rng.normal(s) * 0.05)(S, S)), 'b_sp': _w(1.0 + 0.01 * (lambda *s: _rng.normal(s) * 0.05)(S)), 'w_out': _w((lambda *s: _rng.normal(s) * 0.05)(Fh, D))}
    _B_in = _B_setup()
    return {'A_x': _A_in['x'], 'A_wqkv': _A_in['wqkv'], 'A_w_phi': _A_in['w_phi'], 'A_wo': _A_in['wo'], 'B_x': _B_in['x'], 'B_w_in': _B_in['w_in'], 'B_w_sp': _B_in['w_sp'], 'B_b_sp': _B_in['b_sp'], 'B_w_out': _B_in['w_out']}

def _fwd_reference(A_x, A_wqkv, A_w_phi, A_wo, B_x, B_w_in, B_w_sp, B_b_sp, B_w_out):

    def _A_ref(x, wqkv, w_phi, wo):
        B, S, D = x.shape
        H = 32
        Dh = D // H
        qkv = (lambda x, *d: x.transpose(*d))((x @ wqkv).reshape(B, S, 3, H, Dh), 2, 0, 3, 1, 4)
        q, k, v = (qkv[0], qkv[1], qkv[2])
        pq = jnp.einsum('bhsd,hdf->bhsf', q, w_phi)
        pk = jnp.einsum('bhsd,hdf->bhsf', k, w_phi)
        phi_q = jnp.concatenate([_softmax(pq, axis=-1), _softmax(-pq, axis=-1)], axis=-1)
        phi_k = jnp.concatenate([_softmax(pk, axis=-1), _softmax(-pk, axis=-1)], axis=-1)
        kv = jnp.einsum('bhsf,bhsd->bhfd', phi_k, v)
        z = jnp.einsum('bhsf->bhf', phi_k)
        num = jnp.einsum('bhqf,bhfd->bhqd', phi_q, kv)
        den = jnp.einsum('bhqf,bhf->bhq', phi_q, z)[..., None] + 1e-06
        o = num / den
        return (lambda x, *d: x.transpose(*d))(o, 0, 2, 1, 3).reshape(B, S, D) @ wo

    def _B_ref(x, w_in, w_sp, b_sp, w_out):
        B, S, D = x.shape
        F = w_in.shape[-1]
        Fh = F // 2
        z = _gelu(jnp.einsum('bsd,df->bsf', x, w_in))
        z1 = z[..., :Fh].copy()
        z2 = _layernorm(z[..., Fh:], axis=-1)
        g = jnp.einsum('ts,bsf->btf', w_sp, z2) + b_sp[None, :, None]
        return jnp.einsum('bsf,fd->bsd', z1 * g, w_out)
    x = A_x
    x = x + _A_ref(_layernorm(x, axis=-1), A_wqkv, A_w_phi, A_wo)
    x = x + _B_ref(_layernorm(x, axis=-1), B_w_in, B_w_sp, B_b_sp, B_w_out)
    x = x + _A_ref(_layernorm(x, axis=-1), A_wqkv, A_w_phi, A_wo)
    x = x + _B_ref(_layernorm(x, axis=-1), B_w_in, B_w_sp, B_b_sp, B_w_out)
    return x

def setup_inputs():
    _inp = _fwd_setup_inputs()
    _gk = jax.random.fold_in(jax.random.key(int.from_bytes(__import__("os").urandom(4), "little")), 2 ** 31 - 1)
    _shapes = [[1, 2048, 640]]
    _dtypes = ['bfloat16']
    _gks = jax.random.split(_gk, len(_shapes))
    _gs = [jax.random.normal(k, s, dtype=jnp.dtype(d)) * 0.05 for k, s, d in zip(_gks, _shapes, _dtypes)]
    _inp['grad_out'] = _gs[0]
    return _inp

def reference(A_x, A_wqkv, A_w_phi, A_wo, B_w_in, B_w_sp, B_b_sp, B_w_out, B_x, grad_out):
    _const = dict(B_x=B_x)

    def _f(*_d):
        return _fwd_reference(**{'A_x': _d[0], 'A_wqkv': _d[1], 'A_w_phi': _d[2], 'A_wo': _d[3], 'B_w_in': _d[4], 'B_w_sp': _d[5], 'B_b_sp': _d[6], 'B_w_out': _d[7], **_const})
    _out, _vjp = jax.vjp(_f, A_x, A_wqkv, A_w_phi, A_wo, B_w_in, B_w_sp, B_b_sp, B_w_out)
    _grads = _vjp(grad_out)
    _out0 = jnp.asarray(_out)
    return (_out0, *[jnp.asarray(_g) for _g in _grads])
```

```python
import jax
import jax.numpy as jnp
import jax.experimental.pallas as pl
import jax.experimental.pallas.tpu as pltpu

S, D, H, DH, FH = 2048, 640, 32, 20, 768
NG = 4
GW = 160
GA = 176
N = 256
NC = S // N
F32, BF = jnp.float32, jnp.bfloat16
NT = (((1,), (1,)), ((), ()))
GC, GA3 = 0.7978845608028654, 0.044715


def _nn(a, b):
    return jnp.dot(a, b, preferred_element_type=F32)


def _nt(a, b):
    return jax.lax.dot_general(a, b, NT, preferred_element_type=F32)


def _iota(shape, dim):
    return jax.lax.broadcasted_iota(jnp.int32, shape, dim)


def _div(i, c):
    return jnp.floor((i.astype(F32) + 0.5) * (1.0 / c)).astype(jnp.int32)


def _grouped(i):
    hg = _div(i, GW)
    r = i - hg * GW
    return hg * 8 + (r & 7), r >> 3


def _ln(x):
    mu = jnp.mean(x, axis=0, keepdims=True)
    xc = x - mu
    var = jnp.mean(xc * xc, axis=0, keepdims=True)
    r = jax.lax.rsqrt(var + 1e-5)
    return xc * r, r


def _ln_bwd(dh, h, r):
    m1 = jnp.mean(dh, axis=0, keepdims=True)
    m2 = jnp.mean(dh * h, axis=0, keepdims=True)
    return r * (dh - m1 - h * m2)


def _hedgehog(p):
    n = p.shape[1]
    p3 = p.reshape(DH, 8, n)
    mx = jnp.max(p3, axis=0, keepdims=True)
    mn = jnp.min(p3, axis=0, keepdims=True)
    ep = jnp.exp(p3 - mx)
    en = jnp.exp(mn - p3)
    ep = ep * (1.0 / jnp.sum(ep, axis=0, keepdims=True))
    en = en * (1.0 / jnp.sum(en, axis=0, keepdims=True))
    return ep.reshape(GW, n).astype(BF), en.reshape(GW, n).astype(BF)


def _hedgehog_bwd(dphi, phi):
    n = dphi.shape[1]
    ph = phi.astype(F32).reshape(2, DH, 8, n)
    t = ph * dphi.reshape(2, DH, 8, n)
    sm = jnp.sum(t, axis=1, keepdims=True)
    dp = t - ph * sm
    return (dp[0] - dp[1]).reshape(GW, n)


def _loop(body):
    def f(i, c):
        body(pl.ds(pl.multiple_of(i * N, N), N))
        return c
    jax.lax.fori_loop(0, NC, f, 0)


def _kernel(x_hbm, wqkv_hbm, phi_ref, wo_hbm, win_hbm, wsp_hbm, b_ref, wout_hbm, go_hbm,
            out_hbm, gx_hbm, dwqkv_hbm, dphi_ref, dwo_hbm, dwin_hbm, dwsp_hbm, db_ref, dwout_hbm,
            wsp, WT, W2, woP, woPT, win, winT, wout, woutT, BmT, PmT,
            X, dW2, dwoP, dwin, dwout, dbacc,
            hA1, pq1, pk1, va1, o1, hB1, big1, z2n1, st1, kv1,
            z2n2, dgt2, sems):
    E = (_grouped(_iota((DH, D), 1))[1] == _iota((DH, D), 0)).astype(BF)

    def setup(xin, wq, wo_v):
        cps = [pltpu.make_async_copy(s, d, sems.at[i]) for i, (s, d) in enumerate(
            [(wqkv_hbm, wq), (x_hbm, xin), (wo_hbm, wo_v), (win_hbm, win), (wout_hbm, wout), (wsp_hbm, wsp)])]
        for c in cps:
            c.start()
        T = _nn(phi_ref[...], E)
        hc, _ = _grouped(_iota((D, D), 1))
        BmT[...] = jnp.where(_div(_iota((D, D), 0), DH) == hc, T, 0.0).astype(BF)
        hc, fc = _grouped(_iota((D, D), 1))
        PmT[...] = (_iota((D, D), 0) == hc * DH + fc).astype(BF)
        cps[0].wait()
        for i, m in enumerate((BmT, BmT, PmT)):
            w = _nn(wq[:, i * D:(i + 1) * D], m[...])
            W2[:, i * D:(i + 1) * D] = w.astype(BF)
            WT[i * D:(i + 1) * D, :] = w.T.astype(BF)
        cps[1].wait()

        def tx(c):
            X[:, c] = xin[c, :].astype(F32).T
        _loop(tx)
        cps[2].wait()
        w = _nn(PmT[...].astype(F32).T.astype(BF), wo_v[...])
        woP[...] = w.astype(BF)
        woPT[...] = w.T.astype(BF)
        cps[3].wait()
        winT[...] = win[...].astype(F32).T.astype(BF)
        cps[4].wait()
        woutT[...] = wout[...].astype(F32).T.astype(BF)
        cps[5].wait()

    pl.run_scoped(setup, pltpu.VMEM((S, D), BF), pltpu.VMEM((D, 3 * D), BF), pltpu.VMEM((D, D), BF))

    ones_rows = (_iota((16, N), 0) < 8).astype(BF)
    kvmask = ((_iota((GA, 2 * GW), 0) & 7) == (_iota((GA, 2 * GW), 1) & 7)) & (_iota((GA, 2 * GW), 0) < GW + 8)

    Z1, G, DNA = 1536, 2304, 1920

    def a1(c, x, hA, pq, pk, va, st):
        h, r = _ln(x)
        hb = h.astype(BF)
        hA[:, c] = hb
        st[0:1, c] = r
        p = _nn(WT[...], hb)
        for t, dst in enumerate((pq, pk)):
            for g in range(NG):
                ep, en = _hedgehog(p[t * D + g * GW:t * D + (g + 1) * GW])
                dst[g * 320:g * 320 + GW, c] = ep
                dst[g * 320 + GW:(g + 1) * 320, c] = en
        for g in range(NG):
            va[g * GA:g * GA + GW, c] = p[2 * D + g * GW:2 * D + (g + 1) * GW].astype(BF)
            va[g * GA + GW:(g + 1) * GA, c] = ones_rows

    def kvall(lhs, off, rhs, kv):
        for g in range(NG):
            m = _nt(lhs[off + g * GA:off + (g + 1) * GA, :], rhs[g * 320:(g + 1) * 320, :])
            m = jnp.where(kvmask, m, 0.0)
            kv[g, 0:GA, :] = m.astype(BF)
            kv[g, GA:GA + 320, 0:GA] = m.T.astype(BF)

    def a2(c, pq, o, st, kv):
        os_ = []
        for g in range(NG):
            na = _nn(kv[g, 0:GA, :], pq[g * 320:(g + 1) * 320, c])
            rd = 1.0 / (na[GW:GW + 8] + 1e-6)
            st[8 + g * 8:16 + g * 8, c] = rd
            os_.append((na[0:GW].reshape(DH, 8, N) * rd).reshape(GW, N).astype(BF))
        ob = jnp.concatenate(os_, axis=0)
        o[:, c] = ob
        return X[:, c] + _nn(woPT[...], ob)

    def b1(c, x, hB, big, z2n, st):
        h, r = _ln(x)
        hb = h.astype(BF)
        hB[:, c] = hb
        st[1:2, c] = r
        u = _nn(winT[...], hb)
        u2 = u * u
        t = jnp.tanh(u * (GC + (GC * GA3) * u2))
        ht = 0.5 * t + 0.5
        z = u * ht
        gp = ht + (u * (1.0 - t * t)) * (0.5 * GC + (1.5 * GC * GA3) * u2)
        big[0:2 * FH, c] = gp.astype(BF)
        big[Z1:Z1 + FH, c] = z[0:FH].astype(BF)
        zn, r2 = _ln(z[FH:])
        z2n[:, c] = zn.astype(BF)
        st[2:3, c] = r2

    def b2(c, big, z2n):
        g = _nt(z2n[...], wsp[c, :]) + b_ref[:, c].astype(F32)
        gb = g.astype(BF)
        big[G:G + FH, c] = gb
        y = (big[Z1:Z1 + FH, c].astype(F32) * g).astype(BF)
        return X[:, c] + _nn(woutT[...], y)

    def b2_bwd(c, dxb_c, big, dgt, first):
        dy = _nn(wout[...], dxb_c)
        z1 = big[Z1:Z1 + FH, c].astype(F32)
        g = big[G:G + FH, c].astype(F32)
        dg = dy * z1
        big[Z1:Z1 + FH, c] = (z1 * g).astype(BF)
        big[G:G + FH, c] = dg.astype(BF)
        dgt[c, :] = dg.T.astype(BF)
        big[0:FH, c] = (dy * g * big[0:FH, c].astype(F32)).astype(BF)
        s = jnp.sum(dg, axis=0, keepdims=True)
        dbacc[:, c] = s if first else dbacc[:, c] + s

    def wg(acc, lhs, rhs, first, blk):
        def f(i, cv):
            r = pl.ds(pl.multiple_of(i * blk, blk), blk)
            v = _nt(lhs[r, :], rhs[...])
            acc[r, :] = v if first else acc[r, :] + v
            return cv
        jax.lax.fori_loop(0, lhs.shape[0] // blk, f, 0)

    def b1_bwd(c, hB, big, z2n, st):
        dzn = _nn(big[G:G + FH, :], wsp[:, c])
        dz2 = _ln_bwd(dzn, z2n[:, c].astype(F32), st[2:3, c])
        big[FH:2 * FH, c] = (dz2 * big[FH:2 * FH, c].astype(F32)).astype(BF)
        dh = _nn(win[...], big[0:2 * FH, c])
        return X[:, c] + _ln_bwd(dh, hB[:, c].astype(F32), st[1:2, c])

    def a2_bwd(c, dxb_c, big, pq, o, st, kv):
        do = _nn(woP[...], dxb_c)
        for g in range(NG):
            rd = st[8 + g * 8:16 + g * 8, c]
            dg3 = do[g * GW:(g + 1) * GW].reshape(DH, 8, N)
            o3 = o[g * GW:(g + 1) * GW, c].astype(F32).reshape(DH, 8, N)
            dden = -rd * jnp.sum(dg3 * o3, axis=0)
            dna = jnp.concatenate([(dg3 * rd).reshape(GW, N), dden, jnp.zeros((8, N), F32)], axis=0).astype(BF)
            big[DNA + g * GA:DNA + (g + 1) * GA, c] = dna
            dphi = _nn(kv[g, GA:GA + 320, 0:GA], dna)
            big[g * GW:(g + 1) * GW, c] = _hedgehog_bwd(dphi, pq[g * 320:(g + 1) * 320, c]).astype(BF)

    def a1_bwd(c, big, hA, pk, va, st, kv):
        for g in range(NG):
            ph = pk[g * 320:(g + 1) * 320, c]
            dphi = _nn(kv[g, GA:GA + 320, 0:GA], va[g * GA:(g + 1) * GA, c])
            big[D + g * GW:D + (g + 1) * GW, c] = _hedgehog_bwd(dphi, ph).astype(BF)
            big[2 * D + g * GW:2 * D + (g + 1) * GW, c] = _nn(kv[g, 0:GW, :], ph).astype(BF)
        dh = _nn(W2[...], big[0:3 * D, c])
        return X[:, c] + _ln_bwd(dh, hA[:, c].astype(F32), st[0:1, c])

    def layer_bwd(dxb, hA, pq, pk, va, o, hB, big, z2n, st, kv, first, tail):
        wg(dwout, big.at[Z1:Z1 + FH], dxb, first, 256)

        def p6(c):
            X[:, c] = b1_bwd(c, hB, big, z2n, st)
        _loop(p6)
        wg(dwin, hB, big.at[0:2 * FH], first, 128)

        def p6b(c):
            dxc = X[:, c].astype(BF)
            dxb[:, c] = dxc
            a2_bwd(c, dxc, big, pq, o, st, kv)
        _loop(p6b)
        wg(dwoP, o, dxb, first, 128)
        kvall(big, DNA, pq, kv)

        def p7(c):
            tail(c, a1_bwd(c, big, hA, pk, va, st, kv))
        _loop(p7)
        wg(dW2, hA, big.at[0:3 * D], first, 128)

    _loop(lambda c: a1(c, X[:, c], hA1, pq1, pk1, va1, st1))
    kvall(va1, 0, pk1, kv1)

    def p2(c):
        x = a2(c, pq1, o1, st1, kv1)
        X[:, c] = x
        b1(c, x, hB1, big1, z2n1, st1)
    _loop(p2)

    def layer2(hA2, pq2, pk2, va2, o2, hB2, big2, st2, kv2, dxb, stage):
        gcp = pltpu.make_async_copy(go_hbm, stage, sems.at[0])
        gcp.start()

        def p3(c):
            x = b2(c, big1, z2n1)
            X[:, c] = x
            a1(c, x, hA2, pq2, pk2, va2, st2)
        _loop(p3)
        kvall(va2, 0, pk2, kv2)

        def p4(c):
            x = a2(c, pq2, o2, st2, kv2)
            X[:, c] = x
            b1(c, x, hB2, big2, z2n2, st2)
        _loop(p4)
        gcp.wait()

        def p5(c):
            x = b2(c, big2, z2n2)
            go = stage[c, :].astype(F32).T
            stage[c, :] = x.T.astype(BF)
            X[:, c] = go
            gob = go.astype(BF)
            dxb[:, c] = gob
            b2_bwd(c, gob, big2, dgt2, True)
        _loop(p5)
        ocp = pltpu.make_async_copy(stage, out_hbm, sems.at[1])
        ocp.start()

        def tail(c, dx):
            X[:, c] = dx
        layer_bwd(dxb, hA2, pq2, pk2, va2, o2, hB2, big2, z2n2, st2, kv2, True, tail)
        ocp.wait()

    lay = lambda: [pltpu.VMEM((D, S), BF), pltpu.VMEM((2 * D, S), BF), pltpu.VMEM((2 * D, S), BF),
                   pltpu.VMEM((NG * GA, S), BF), pltpu.VMEM((D, S), BF), pltpu.VMEM((D, S), BF),
                   pltpu.VMEM((4 * FH, S), BF), pltpu.VMEM((40, S), F32), pltpu.VMEM((NG, GA + 320, 320), BF)]
    pl.run_scoped(layer2, *lay(), pltpu.VMEM((D, S), BF), pltpu.VMEM((S, D), BF))

    def layer1(dxb, dgt1, stage, spst, wq, s_qkv, s_wo, s_win, s_wout):
        wcp = pltpu.make_async_copy(wqkv_hbm, wq, sems.at[0])
        wcp.start()

        def p7b(c):
            dxc = X[:, c].astype(BF)
            dxb[:, c] = dxc
            b2_bwd(c, dxc, big1, dgt1, False)
        _loop(p7b)

        def psp(c):
            spst[c, :] = (_nn(dgt1[c, :], z2n1[...]) + _nn(dgt2[c, :], z2n2[...])).astype(BF)
        _loop(psp)
        c1 = pltpu.make_async_copy(spst, dwsp_hbm, sems.at[1])
        c1.start()
        db_ref[...] = dbacc[...].astype(BF)

        def tail(c, dx):
            stage[c, :] = dx.T.astype(BF)
        layer_bwd(dxb, hA1, pq1, pk1, va1, o1, hB1, big1, z2n1, st1, kv1, False, tail)
        c2 = pltpu.make_async_copy(stage, gx_hbm, sems.at[2])
        c2.start()
        s_win[...] = dwin[...].astype(BF)
        s_wout[...] = dwout[...].astype(BF)
        c3 = pltpu.make_async_copy(s_win, dwin_hbm, sems.at[3])
        c4 = pltpu.make_async_copy(s_wout, dwout_hbm, sems.at[4])
        c3.start()
        c4.start()
        s_wo[...] = _nn(PmT[...], dwoP[...].astype(BF)).astype(BF)
        c5 = pltpu.make_async_copy(s_wo, dwo_hbm, sems.at[5])
        c5.start()
        for i, m in enumerate((BmT, BmT, PmT)):
            s_qkv[:, i * D:(i + 1) * D] = _nt(dW2[:, i * D:(i + 1) * D].astype(BF), m[...]).astype(BF)
        c6 = pltpu.make_async_copy(s_qkv, dwqkv_hbm, sems.at[6])
        c6.start()
        wcp.wait()
        acc = (_nn(wq[:, 0:D].astype(F32).T.astype(BF), dW2[:, 0:D].astype(BF))
               + _nn(wq[:, D:2 * D].astype(F32).T.astype(BF), dW2[:, D:2 * D].astype(BF)))
        hc, _ = _grouped(_iota((D, D), 1))
        acc = jnp.where(_div(_iota((D, D), 0), DH) == hc, acc, 0.0).astype(BF)
        dphi_ref[...] = _nt(acc, E).astype(BF)
        for c in (c1, c2, c3, c4, c5, c6):
            c.wait()

    pl.run_scoped(layer1, pltpu.VMEM((D, S), BF), pltpu.VMEM((S, FH), BF), pltpu.VMEM((S, D), BF),
                  pltpu.VMEM((S, S), BF), pltpu.VMEM((D, 3 * D), BF), pltpu.VMEM((D, 3 * D), BF),
                  pltpu.VMEM((D, D), BF), pltpu.VMEM((D, 2 * FH), BF), pltpu.VMEM((FH, D), BF))


@jax.jit
def pallas_interleave_layers__linear_kernel_hedgehog__mixer_gmlp__prompt_kernel(
    A_x: jax.Array,
    A_wqkv: jax.Array,
    A_w_phi: jax.Array,
    A_wo: jax.Array,
    B_x: jax.Array,
    B_w_in: jax.Array,
    B_w_sp: jax.Array,
    B_b_sp: jax.Array,
    B_w_out: jax.Array,
    grad_out: jax.Array,
):
    del B_x
    hbm = pl.BlockSpec(memory_space=pl.ANY)
    vm = pl.BlockSpec(memory_space=pltpu.VMEM)
    V = pltpu.VMEM
    sd = jax.ShapeDtypeStruct
    scratch = [
        V((S, S), BF), V((3 * D, D), BF), V((D, 3 * D), BF), V((D, D), BF), V((D, D), BF),
        V((D, 2 * FH), BF), V((2 * FH, D), BF), V((FH, D), BF), V((D, FH), BF), V((D, D), BF), V((D, D), BF),
        V((D, S), F32), V((D, 3 * D), F32), V((D, D), F32), V((D, 2 * FH), F32), V((FH, D), F32), V((1, S), F32),
        V((D, S), BF), V((2 * D, S), BF), V((2 * D, S), BF), V((NG * GA, S), BF), V((D, S), BF), V((D, S), BF),
        V((4 * FH, S), BF), V((FH, S), BF), V((40, S), F32), V((NG, GA + 320, 320), BF),
        V((FH, S), BF), V((S, FH), BF), pltpu.SemaphoreType.DMA((8,)),
    ]
    outs = pl.pallas_call(
        _kernel,
        in_specs=[hbm, hbm, vm, hbm, hbm, hbm, vm, hbm, hbm],
        out_specs=[hbm, hbm, hbm, vm, hbm, hbm, hbm, vm, hbm],
        out_shape=[sd((S, D), BF), sd((S, D), BF), sd((D, 3 * D), BF), sd((D, DH), BF), sd((D, D), BF),
                   sd((D, 2 * FH), BF), sd((S, S), BF), sd((1, S), BF), sd((FH, D), BF)],
        scratch_shapes=scratch,
        compiler_params=pltpu.CompilerParams(vmem_limit_bytes=128 * 2**20),
    )(A_x.reshape(S, D), A_wqkv, A_w_phi.reshape(D, DH), A_wo, B_w_in, B_w_sp, B_b_sp.reshape(1, S),
      B_w_out, grad_out.reshape(S, D))
    out, gx, dwqkv, dphi, dwo, dwin, dwsp, db, dwout = outs
    return (out.reshape(1, S, D), gx.reshape(1, S, D), dwqkv, dphi.reshape(H, DH, DH), dwo, dwin, dwsp,
            db.reshape(S), dwout)
```

```python
import jax
import jax.numpy as jnp
import jax.experimental.pallas as pl
import jax.experimental.pallas.tpu as pltpu

S, D, H, DH, FH = 2048, 640, 32, 20, 768
NG = 4
GW = 160
GA = 176
N = 256
NSUB = 1
NC = S // (N * NSUB)
F32, BF = jnp.float32, jnp.bfloat16
NT = (((1,), (1,)), ((), ()))
GC, GA3 = 0.7978845608028654, 0.044715


def _nn(a, b):
    return jnp.dot(a, b, preferred_element_type=F32)


def _mm(w, b):
    m, k = w.shape
    if (-(-k // 128) * (b.shape[1] // 128)) % 4 == 2:
        return jnp.concatenate([_nn(w[0:m // 2, :], b), _nn(w[m // 2:m, :], b)], axis=0)
    return _mm(w, b)


def _nt(a, b):
    return jax.lax.dot_general(a, b, NT, preferred_element_type=F32)


def _iota(shape, dim):
    return jax.lax.broadcasted_iota(jnp.int32, shape, dim)


def _div(i, c):
    return jnp.floor((i.astype(F32) + 0.5) * (1.0 / c)).astype(jnp.int32)


def _grouped(i):
    hg = _div(i, GW)
    r = i - hg * GW
    return hg * 8 + (r & 7), r >> 3


def _ln(x):
    mu = jnp.mean(x, axis=0, keepdims=True)
    xc = x - mu
    var = jnp.mean(xc * xc, axis=0, keepdims=True)
    r = jax.lax.rsqrt(var + 1e-5)
    return xc * r, r


def _ln_bwd(dh, h, r):
    m1 = jnp.mean(dh, axis=0, keepdims=True)
    m2 = jnp.mean(dh * h, axis=0, keepdims=True)
    return r * (dh - m1 - h * m2)


def _hedgehog(p):
    n = p.shape[1]
    p3 = p.reshape(DH, 8, n)
    mx = jnp.max(p3, axis=0, keepdims=True)
    mn = jnp.min(p3, axis=0, keepdims=True)
    ep = jnp.exp(p3 - mx)
    en = jnp.exp(mn - p3)
    ep = ep * (1.0 / jnp.sum(ep, axis=0, keepdims=True))
    en = en * (1.0 / jnp.sum(en, axis=0, keepdims=True))
    return ep.reshape(GW, n).astype(BF), en.reshape(GW, n).astype(BF)


def _hedgehog_bwd(dphi, phi):
    n = dphi.shape[1]
    ph = phi.astype(F32).reshape(2, DH, 8, n)
    t = ph * dphi.reshape(2, DH, 8, n)
    sm = jnp.sum(t, axis=1, keepdims=True)
    dp = t - ph * sm
    return (dp[0] - dp[1]).reshape(GW, n)


def _loop(body, name=None):
    def f(i, c):
        gens = [body(pl.ds(pl.multiple_of((i * NSUB + k) * N, N), N)) for k in range(NSUB)]
        while gens:
            gens = [g for g in gens if next(g, 0) is None]
        return c
    with jax.named_scope(name or body.__name__):
        jax.lax.fori_loop(0, NC, f, 0)


def _drain(g):
    try:
        while True:
            next(g)
    except StopIteration as e:
        return e.value


def _skew(head, tail, ubuf, name, mid=None):
    stages = [lambda c, v: _drain(head(c))] + ([mid] if mid else []) + [tail]
    ns = len(stages)
    rows = [0] * ns
    offs = [0, 0, D]

    def step(t, lo, hi):
        ks = range(lo, hi)
        vs = [ubuf[offs[k]:offs[k] + rows[k], :] if rows[k] else None for k in ks]
        res = [stages[k](pl.ds(pl.multiple_of((t - k) * N, N), N), v) for k, v in zip(ks, vs)]
        for k, r in zip(ks, res):
            if k + 1 < ns and r is not None:
                rows[k + 1] = r.shape[0]
                if k == 0 and ns == 3:
                    offs[2] = rows[1]
                ubuf[offs[k + 1]:offs[k + 1] + r.shape[0], :] = r
            elif k == 0:
                offs[2] = 0

    with jax.named_scope(name):
        for t in range(ns - 1):
            step(t, 0, t + 1)

        def f(t, cv):
            step(t, 0, ns)
            return cv
        jax.lax.fori_loop(ns - 1, NC, f, 0)
        for t in range(NC, NC + ns - 1):
            step(t, t - NC + 1, ns)


def _kernel(x_hbm, wqkv_hbm, phi_ref, wo_hbm, win_hbm, wsp_hbm, b_ref, wout_hbm, go_hbm,
            out_hbm, gx_hbm, dwqkv_hbm, dphi_ref, dwo_hbm, dwin_hbm, dwsp_hbm, db_ref, dwout_hbm, pk_hbm, va_hbm,
            wsp, WT, W2, woP, woPT, win, winT, wout, woutT, BmT, PmT,
            X, dW2, dwoP, dwin, dwout, dbacc,
            hA1, pq1, pk1, va1, o1, hB1, big1, z2n1, st1, kv1,
            z2n2, dgt2, ubuf, sems):
    E = (_grouped(_iota((DH, D), 1))[1] == _iota((DH, D), 0)).astype(BF)

    def setup(xin, wq, wo_v):
        cps = [pltpu.make_async_copy(s, d, sems.at[i]) for i, (s, d) in enumerate(
            [(wqkv_hbm, wq), (x_hbm, xin), (wo_hbm, wo_v), (win_hbm, win), (wout_hbm, wout), (wsp_hbm, wsp)])]
        for c in cps:
            c.start()
        T = _nn(phi_ref[...], E)
        hc, _ = _grouped(_iota((D, D), 1))
        BmT[...] = jnp.where(_div(_iota((D, D), 0), DH) == hc, T, 0.0).astype(BF)
        hc, fc = _grouped(_iota((D, D), 1))
        PmT[...] = (_iota((D, D), 0) == hc * DH + fc).astype(BF)
        cps[0].wait()
        for i, m in enumerate((BmT, BmT, PmT)):
            w = _nn(wq[:, i * D:(i + 1) * D], m[...])
            W2[:, i * D:(i + 1) * D] = w.astype(BF)
            WT[i * D:(i + 1) * D, :] = w.T.astype(BF)
        cps[1].wait()

        def tx(c):
            X[:, c] = xin[c, :].astype(F32).T
            yield
        _loop(tx)
        cps[2].wait()
        w = _nn(PmT[...].astype(F32).T.astype(BF), wo_v[...])
        woP[...] = w.astype(BF)
        woPT[...] = w.T.astype(BF)
        cps[3].wait()
        winT[...] = win[...].astype(F32).T.astype(BF)
        cps[4].wait()
        woutT[...] = wout[...].astype(F32).T.astype(BF)

    with jax.named_scope("setup"):
      pl.run_scoped(setup, pltpu.VMEM((S, D), BF), pltpu.VMEM((D, 3 * D), BF), pltpu.VMEM((D, D), BF))

    ones_rows = (_iota((16, N), 0) < 8).astype(BF)
    kvmask = ((_iota((GA, 2 * GW), 0) & 7) == (_iota((GA, 2 * GW), 1) & 7)) & (_iota((GA, 2 * GW), 0) < GW + 8)

    Z1, G, DNA = 1536, 2304, 1920

    def a1(c, x, hA, st):
        h, r = _ln(x)
        hb = h.astype(BF)
        hA[:, c] = hb
        st[0:1, c] = r
        return _mm(WT, hb)

    def a1t(c, p, pq, pk, va):
        for t, dst in enumerate((pq, pk)):
            for g in range(NG):
                ep, en = _hedgehog(p[t * D + g * GW:t * D + (g + 1) * GW])
                dst[g * 320:g * 320 + GW, c] = ep
                dst[g * 320 + GW:(g + 1) * 320, c] = en
        for g in range(NG):
            va[g * GA:g * GA + GW, c] = p[2 * D + g * GW:2 * D + (g + 1) * GW].astype(BF)
            va[g * GA + GW:(g + 1) * GA, c] = ones_rows

    def kvall(lhs, off, rhs, kv):
      with jax.named_scope("kvall"):
        for g in range(NG):
            m = _nt(lhs[off + g * GA:off + (g + 1) * GA, :], rhs[g * 320:(g + 1) * 320, :])
            m = jnp.where(kvmask, m, 0.0)
            kv[g, 0:GA, :] = m.astype(BF)
            kv[g, GA:GA + 320, 0:GA] = m.T.astype(BF)

    def a2(c, pq, o, st, kv):
        os_ = []
        for g in range(NG):
            na = _nn(kv[g, 0:GA, :], pq[g * 320:(g + 1) * 320, c])
            rd = 1.0 / (na[GW:GW + 8] + 1e-6)
            st[8 + g * 8:16 + g * 8, c] = rd
            os_.append((na[0:GW].reshape(DH, 8, N) * rd).reshape(GW, N).astype(BF))
        ob = jnp.concatenate(os_, axis=0)
        o[:, c] = ob
        yield
        return X[:, c] + _mm(woPT, ob)

    def b1(c, x, hB, st):
        h, r = _ln(x)
        hb = h.astype(BF)
        hB[:, c] = hb
        st[1:2, c] = r
        return _mm(winT, hb)

    def b1t(c, u, big, z2n, st):
        u2 = u * u
        t = jnp.tanh(u * (GC + (GC * GA3) * u2))
        ht = 0.5 * t + 0.5
        z = u * ht
        gp = ht + (u * (1.0 - t * t)) * (0.5 * GC + (1.5 * GC * GA3) * u2)
        big[0:2 * FH, c] = gp.astype(BF)
        big[Z1:Z1 + FH, c] = z[0:FH].astype(BF)
        zn, r2 = _ln(z[FH:])
        z2n[:, c] = zn.astype(BF)
        st[2:3, c] = r2

    def b2(c, big, z2n):
        g = _nt(z2n[...], wsp[c, :]) + b_ref[:, c].astype(F32)
        yield
        gb = g.astype(BF)
        big[G:G + FH, c] = gb
        y = (big[Z1:Z1 + FH, c].astype(F32) * g).astype(BF)
        return X[:, c] + _nn(woutT[...], y)

    def b2_bwd(c, dy, big, dgt, first):
        z1 = big[Z1:Z1 + FH, c].astype(F32)
        g = big[G:G + FH, c].astype(F32)
        dg = dy * z1
        big[Z1:Z1 + FH, c] = (z1 * g).astype(BF)
        big[G:G + FH, c] = dg.astype(BF)
        dgt[c, :] = dg.T.astype(BF)
        big[0:FH, c] = (dy * g * big[0:FH, c].astype(F32)).astype(BF)
        s = jnp.sum(dg, axis=0, keepdims=True)
        dbacc[:, c] = s if first else dbacc[:, c] + s

    def wg(acc, lhs, rhs, first, blk):
        def f(i, cv):
            r = pl.ds(pl.multiple_of(i * blk, blk), blk)
            v = _nt(lhs[r, :], rhs[...])
            acc[r, :] = v if first else acc[r, :] + v
            return cv
        with jax.named_scope("wg_%d_%d_%d" % (lhs.shape[0], rhs.shape[0], first)):
            jax.lax.fori_loop(0, lhs.shape[0] // blk, f, 0)

    def b1_bwd(c, hB, big, z2n, st):
        dzn = _nn(big[G:G + FH, :], wsp[:, c])
        yield
        return dzn

    def b1_bwd2(c, dzn, big, z2n, st):
        dz2 = _ln_bwd(dzn, z2n[:, c].astype(F32), st[2:3, c])
        big[FH:2 * FH, c] = (dz2 * big[FH:2 * FH, c].astype(F32)).astype(BF)
        return _nn(win[...], big[0:2 * FH, c])

    def a2_bwd(c, do, big, pq, o, st, kv):
        for g in range(NG):
            rd = st[8 + g * 8:16 + g * 8, c]
            dg3 = do[g * GW:(g + 1) * GW].reshape(DH, 8, N)
            o3 = o[g * GW:(g + 1) * GW, c].astype(F32).reshape(DH, 8, N)
            dden = -rd * jnp.sum(dg3 * o3, axis=0)
            dna = jnp.concatenate([(dg3 * rd).reshape(GW, N), dden, jnp.zeros((8, N), F32)], axis=0).astype(BF)
            big[DNA + g * GA:DNA + (g + 1) * GA, c] = dna
            dphi = _nn(kv[g, GA:GA + 320, 0:GA], dna)
            big[g * GW:(g + 1) * GW, c] = _hedgehog_bwd(dphi, pq[g * 320:(g + 1) * 320, c]).astype(BF)

    def a1_bwd(c, big, hA, pk, va, st, kv):
        for g in range(NG):
            ph = pk[g * 320:(g + 1) * 320, c]
            dphi = _nn(kv[g, GA:GA + 320, 0:GA], va[g * GA:(g + 1) * GA, c])
            big[D + g * GW:D + (g + 1) * GW, c] = _hedgehog_bwd(dphi, ph).astype(BF)
            big[2 * D + g * GW:2 * D + (g + 1) * GW, c] = _nn(kv[g, 0:GW, :], ph).astype(BF)
        yield
        return _mm(W2, big[0:3 * D, c])

    def castmm(c, dxb, w):
        dxc = X[:, c].astype(BF)
        dxb[:, c] = dxc
        yield
        return _mm(w, dxc)

    def layer_bwd(dxb, hA, pq, pk, va, o, hB, big, z2n, st, kv, first, tail, early=lambda: None):
        wg(dwout, big.at[Z1:Z1 + FH], dxb, first, 256)

        def p6t(c, dh):
            X[:, c] = X[:, c] + _ln_bwd(dh, hB[:, c].astype(F32), st[1:2, c])
        _skew(lambda c: b1_bwd(c, hB, big, z2n, st), p6t, ubuf, "p6",
              lambda c, v: b1_bwd2(c, v, big, z2n, st))
        wg(dwin, hB, big.at[0:2 * FH], first, 128)

        _skew(lambda c: castmm(c, dxb, woP), lambda c, do: a2_bwd(c, do, big, pq, o, st, kv), ubuf, "p6b")
        wg(dwoP, o, dxb, first, 128)
        early()
        kvall(big, DNA, pq, kv)

        def p7t(c, dh):
            tail(c, X[:, c] + _ln_bwd(dh, hA[:, c].astype(F32), st[0:1, c]))
        _skew(lambda c: a1_bwd(c, big, hA, pk, va, st, kv), p7t, ubuf, "p7")
        wg(dW2, hA, big.at[0:3 * D], first, 128)

    def p1(c):
        yield
        return a1(c, X[:, c], hA1, st1)
    _skew(p1, lambda c, p: a1t(c, p, pq1, pk1, va1), ubuf, "p1")
    kvall(va1, 0, pk1, kv1)
    park = [pltpu.make_async_copy(pk1, pk_hbm, sems.at[6]), pltpu.make_async_copy(va1, va_hbm, sems.at[7])]
    for cp in park:
        cp.start()

    def p2(c):
        x = yield from a2(c, pq1, o1, st1, kv1)
        X[:, c] = x
        yield
        return x
    _skew(p2, lambda c, u: b1t(c, u, big1, z2n1, st1), ubuf, "p2",
          lambda c, v: b1(c, v, hB1, st1))

    for cp in park:
        cp.wait()
    pltpu.make_async_copy(wsp_hbm, wsp, sems.at[5]).wait()
    pk2, va2 = pk1, va1

    def layer2(hA2, pq2, o2, hB2, big2, st2, kv2, dxb, stage):
        gcp = pltpu.make_async_copy(go_hbm, stage, sems.at[0])
        gcp.start()

        def p3(c):
            x = yield from b2(c, big1, z2n1)
            X[:, c] = x
            yield
            return x
        _skew(p3, lambda c, p: a1t(c, p, pq2, pk2, va2), ubuf, "p3",
          lambda c, v: a1(c, v, hA2, st2))
        kvall(va2, 0, pk2, kv2)

        def p4(c):
            x = yield from a2(c, pq2, o2, st2, kv2)
            X[:, c] = x
            yield
            return x
        _skew(p4, lambda c, u: b1t(c, u, big2, z2n2, st2), ubuf, "p4",
          lambda c, v: b1(c, v, hB2, st2))
        gcp.wait()

        def p5(c):
            x = yield from b2(c, big2, z2n2)
            go = stage[c, :].astype(F32).T
            stage[c, :] = x.T.astype(BF)
            X[:, c] = go
            gob = go.astype(BF)
            dxb[:, c] = gob
            yield
            return _mm(wout, gob)
        _skew(p5, lambda c, dy: b2_bwd(c, dy, big2, dgt2, True), ubuf, "p5")
        ocp = pltpu.make_async_copy(stage, out_hbm, sems.at[1])
        ocp.start()

        def tail(c, dx):
            X[:, c] = dx
        layer_bwd(dxb, hA2, pq2, pk2, va2, o2, hB2, big2, z2n2, st2, kv2, True, tail)
        ocp.wait()

    lay = lambda: [pltpu.VMEM((D, S), BF), pltpu.VMEM((2 * D, S), BF),
                   pltpu.VMEM((D, S), BF), pltpu.VMEM((D, S), BF),
                   pltpu.VMEM((4 * FH, S), BF), pltpu.VMEM((40, S), F32), pltpu.VMEM((NG, GA + 320, 320), BF)]
    pl.run_scoped(layer2, *lay(), pltpu.VMEM((D, S), BF), pltpu.VMEM((S, D), BF))

    def layer1(dxb, dgt1, stage, spst, wq, s_qkv, s_wo, s_win, s_wout):
        wcp = pltpu.make_async_copy(wqkv_hbm, wq, sems.at[0])
        wcp.start()
        back = [pltpu.make_async_copy(pk_hbm, pk1, sems.at[6]), pltpu.make_async_copy(va_hbm, va1, sems.at[7])]
        for cp in back:
            cp.start()

        _skew(lambda c: castmm(c, dxb, wout), lambda c, dy: b2_bwd(c, dy, big1, dgt1, False), ubuf, "p7b")

        def psp(c):
            spst[c, :] = (_nn(dgt1[c, :], z2n1[...]) + _nn(dgt2[c, :], z2n2[...])).astype(BF)
            yield
        _loop(psp)
        c1 = pltpu.make_async_copy(spst, dwsp_hbm, sems.at[1])
        c1.start()
        db_ref[...] = dbacc[...].astype(BF)

        for cp in back:
            cp.wait()

        c3 = pltpu.make_async_copy(s_win, dwin_hbm, sems.at[3])
        c4 = pltpu.make_async_copy(s_wout, dwout_hbm, sems.at[4])

        def early():
            s_win[...] = dwin[...].astype(BF)
            s_wout[...] = dwout[...].astype(BF)
            c3.start()
            c4.start()

        def tail(c, dx):
            stage[c, :] = dx.T.astype(BF)
        layer_bwd(dxb, hA1, pq1, pk1, va1, o1, hB1, big1, z2n1, st1, kv1, False, tail, early)
        c2 = pltpu.make_async_copy(stage, gx_hbm, sems.at[2])
        c2.start()
        s_wo[...] = _nn(PmT[...], dwoP[...].astype(BF)).astype(BF)
        c5 = pltpu.make_async_copy(s_wo, dwo_hbm, sems.at[5])
        c5.start()
        for i, m in enumerate((BmT, BmT, PmT)):
            s_qkv[:, i * D:(i + 1) * D] = _nt(dW2[:, i * D:(i + 1) * D].astype(BF), m[...]).astype(BF)
        c6 = pltpu.make_async_copy(s_qkv, dwqkv_hbm, sems.at[6])
        c6.start()
        wcp.wait()
        acc = (_nn(wq[:, 0:D].astype(F32).T.astype(BF), dW2[:, 0:D].astype(BF))
               + _nn(wq[:, D:2 * D].astype(F32).T.astype(BF), dW2[:, D:2 * D].astype(BF)))
        hc, _ = _grouped(_iota((D, D), 1))
        acc = jnp.where(_div(_iota((D, D), 0), DH) == hc, acc, 0.0).astype(BF)
        dphi_ref[...] = _nt(acc, E).astype(BF)
        for c in (c1, c2, c3, c4, c5, c6):
            c.wait()

    pl.run_scoped(layer1, pltpu.VMEM((D, S), BF), pltpu.VMEM((S, FH), BF), pltpu.VMEM((S, D), BF),
                  pltpu.VMEM((S, S), BF), pltpu.VMEM((D, 3 * D), BF), pltpu.VMEM((D, 3 * D), BF),
                  pltpu.VMEM((D, D), BF), pltpu.VMEM((D, 2 * FH), BF), pltpu.VMEM((FH, D), BF))


@jax.jit
def pallas_interleave_layers__linear_kernel_hedgehog__mixer_gmlp__prompt_kernel(
    A_x: jax.Array,
    A_wqkv: jax.Array,
    A_w_phi: jax.Array,
    A_wo: jax.Array,
    B_x: jax.Array,
    B_w_in: jax.Array,
    B_w_sp: jax.Array,
    B_b_sp: jax.Array,
    B_w_out: jax.Array,
    grad_out: jax.Array,
):
    del B_x
    hbm = pl.BlockSpec(memory_space=pl.ANY)
    vm = pl.BlockSpec(memory_space=pltpu.VMEM)
    V = pltpu.VMEM
    sd = jax.ShapeDtypeStruct
    scratch = [
        V((S, S), BF), V((3 * D, D), BF), V((D, 3 * D), BF), V((D, D), BF), V((D, D), BF),
        V((D, 2 * FH), BF), V((2 * FH, D), BF), V((FH, D), BF), V((D, FH), BF), V((D, D), BF), V((D, D), BF),
        V((D, S), F32), V((D, 3 * D), F32), V((D, D), F32), V((D, 2 * FH), F32), V((FH, D), F32), V((1, S), F32),
        V((D, S), BF), V((2 * D, S), BF), V((2 * D, S), BF), V((NG * GA, S), BF), V((D, S), BF), V((D, S), BF),
        V((4 * FH, S), BF), V((FH, S), BF), V((40, S), F32), V((NG, GA + 320, 320), BF),
        V((FH, S), BF), V((S, FH), BF), V((4 * D, N), F32), pltpu.SemaphoreType.DMA((8,)),
    ]
    outs = pl.pallas_call(
        _kernel,
        in_specs=[hbm, hbm, vm, hbm, hbm, hbm, vm, hbm, hbm],
        out_specs=[hbm, hbm, hbm, vm, hbm, hbm, hbm, vm, hbm, hbm, hbm],
        out_shape=[sd((S, D), BF), sd((S, D), BF), sd((D, 3 * D), BF), sd((D, DH), BF), sd((D, D), BF),
                   sd((D, 2 * FH), BF), sd((S, S), BF), sd((1, S), BF), sd((FH, D), BF),
                   sd((2 * D, S), BF), sd((NG * GA, S), BF)],
        scratch_shapes=scratch,
        compiler_params=pltpu.CompilerParams(vmem_limit_bytes=128 * 2**20),
    )(A_x.reshape(S, D), A_wqkv, A_w_phi.reshape(D, DH), A_wo, B_w_in, B_w_sp, B_b_sp.reshape(1, S),
      B_w_out, grad_out.reshape(S, D))
    out, gx, dwqkv, dphi, dwo, dwin, dwsp, db, dwout = outs[:9]
    return (out.reshape(1, S, D), gx.reshape(1, S, D), dwqkv, dphi.reshape(H, DH, DH), dwo, dwin, dwsp,
            db.reshape(S), dwout)
```
